```python
import jax
import jax.numpy as jnp

def _softmax(x, axis=-1):
    return jax.nn.softmax(x, axis=axis)
def _gelu(x):
    return jax.nn.gelu(x, approximate=True)
def _silu(x):
    return jax.nn.silu(x)
def _sigmoid(x):
    return jax.nn.sigmoid(x)
def _layernorm(x, axis=-1, eps=1e-5):
    m = jnp.mean(x, axis=axis, keepdims=True)
    v = jnp.var(x, axis=axis, keepdims=True)
    return (x - m) / jnp.sqrt(v + eps)
def _scatter_add(tgt, idx, src, axis=0):
    return tgt.at[idx].add(src)
def _segment_sum(src, seg, n):
    return jax.ops.segment_sum(src, seg, n)
class _Rng:
    def __init__(self, key):
        self._k = key
    def _next(self):
        self._k, sub = jax.random.split(self._k)
        return sub
    def normal(self, shape):
        return jax.random.normal(self._next(), shape, dtype=jnp.bfloat16)
    def randint(self, lo, hi, shape):
        return jax.random.randint(self._next(), shape, lo, hi, dtype=jnp.int32)
    def uniform(self, shape, lo=0.0, hi=1.0):
        return jax.random.uniform(self._next(), shape, jnp.bfloat16, lo, hi)
    def permutation(self, n):
        return jax.random.permutation(self._next(), n)


kernel_name = 'sequential_preLN__sliding_block__glu_gated_glu__prompt'

def _fwd_setup_inputs():
    _rng = _Rng(jax.random.key(int.from_bytes(__import__("os").urandom(4), "little")))
    _w = (lambda a: (lambda t: t.astype(jnp.bfloat16) if jnp.issubdtype(t.dtype, jnp.floating) else t)(jnp.asarray(a)))
    def _A_setup():
        B, S, D = 1, 2048, 512
        return {
            "x": _w((lambda *s: _rng.normal(s) * 0.05)(B, S, D)),
            "wqkv": _w((lambda *s: _rng.normal(s) * 0.05)(D, 3 * D)),
            "wo": _w((lambda *s: _rng.normal(s) * 0.05)(D, D)),
        }
    _A_in = _A_setup()

    def _B_setup():
        B, S, D, F = 1, 2048, 512, 1376
        return {
            "x": _w((lambda *s: _rng.normal(s) * 0.05)(B, S, D)),
            "w_gate": _w((lambda *s: _rng.normal(s) * 0.05)(D, F)),
            "w_up": _w((lambda *s: _rng.normal(s) * 0.05)(D, F)),
            "w_down": _w((lambda *s: _rng.normal(s) * 0.05)(F, D)),
        }
    _B_in = _B_setup()

    return {
        "A_x": _A_in["x"],
        "A_wqkv": _A_in["wqkv"],
        "A_wo": _A_in["wo"],
        "B_x": _B_in["x"],
        "B_w_gate": _B_in["w_gate"],
        "B_w_up": _B_in["w_up"],
        "B_w_down": _B_in["w_down"],
    }

def _fwd_reference(A_x, A_wqkv, A_wo, B_x, B_w_gate, B_w_up, B_w_down):
    def _A_ref(x, wqkv, wo):
        B, S, D = x.shape
        H = 32; Dh = D // H; W = 256
        qkv = (lambda x, *d: x.transpose(*d))((x @ wqkv).reshape(B, S, 3, H, Dh), 2, 0, 3, 1, 4)
        q, k, v = qkv[0], qkv[1], qkv[2]
        scores = jnp.einsum("bhqd,bhkd->bhqk", q, k) * (Dh ** -0.5)
        idx = jnp.arange(S)
        mask = (idx[:, None] - idx[None, :] >= 0) & (idx[:, None] - idx[None, :] < W)
        scores = jnp.where(mask[None, None], scores, -1e9)
        p = _softmax(scores, axis=-1)
        o = jnp.einsum("bhqk,bhkd->bhqd", p, v)
        return (lambda x, *d: x.transpose(*d))(o, 0, 2, 1, 3).reshape(B, S, D) @ wo

    def _B_ref(x, w_gate, w_up, w_down):
        g = jnp.einsum("bsd,df->bsf", x, w_gate)
        u = jnp.einsum("bsd,df->bsf", x, w_up)
        h = _sigmoid(g) * u
        return jnp.einsum("bsf,fd->bsd", h, w_down)

    x = A_x
    h = x + _A_ref(_layernorm(x, axis=-1), A_wqkv, A_wo)
    h2 = h + _B_ref(_layernorm(h, axis=-1), B_w_gate, B_w_up, B_w_down)
    return h2


def setup_inputs():
    _inp = _fwd_setup_inputs()
    _gk = jax.random.fold_in(jax.random.key(int.from_bytes(__import__("os").urandom(4), "little")), 2**31 - 1)
    _shapes = [[1, 2048, 512]]
    _dtypes = ['bfloat16']
    _gks = jax.random.split(_gk, len(_shapes))
    _gs = [jax.random.normal(k, s, dtype=jnp.dtype(d)) * 0.05 for k, s, d in zip(_gks, _shapes, _dtypes)]
    _inp["grad_out"] = _gs[0]
    return _inp

def reference(A_x, A_wqkv, A_wo, B_w_gate, B_w_up, B_w_down, B_x, grad_out):
    _const = dict(B_x=B_x)
    def _f(*_d):
        return _fwd_reference(**{'A_x': _d[0], 'A_wqkv': _d[1], 'A_wo': _d[2], 'B_w_gate': _d[3], 'B_w_up': _d[4], 'B_w_down': _d[5], **_const})
    _out, _vjp = jax.vjp(_f, A_x, A_wqkv, A_wo, B_w_gate, B_w_up, B_w_down)
    _grads = _vjp(grad_out)
    _out0 = jnp.asarray(_out)
    return (_out0, *[jnp.asarray(_g) for _g in _grads])
```

```python
import math

import jax
import jax.numpy as jnp
import jax.experimental.pallas as pl
import jax.experimental.pallas.tpu as pltpu

S, D, F, H = 2048, 512, 1376, 32
DH = D // H
T = 256
NC = S // T
QB = 128
NB = S // QB
EPS = 1e-5
LOG2E = math.log2(math.e)
SCALE = DH ** -0.5
FC = 352
HU = 8
BF, F32 = jnp.bfloat16, jnp.float32


def _when(cond, name):
    def deco(fn):
        @pl.when(cond)
        def _():
            with jax.named_scope(name):
                fn()
    return deco


def _nn(a, b):
    return jnp.dot(a, b, preferred_element_type=F32)


def _nt(a, b):
    return jax.lax.dot_general(a, b, (((1,), (1,)), ((), ())), preferred_element_type=F32)


def _chunks(n, step):
    return [(i, min(step, n - i)) for i in range(0, n, step)]


def _ln_t(v):
    mu = jnp.mean(v, axis=0, keepdims=True)
    vc = v - mu
    rstd = jax.lax.rsqrt(jnp.mean(vc * vc, axis=0, keepdims=True) + EPS)
    return vc * rstd, rstd


def _ln_bwd_t(dn, xh, rstd):
    m1 = jnp.mean(dn, axis=0, keepdims=True)
    m2 = jnp.mean(dn * xh, axis=0, keepdims=True)
    return rstd * (dn - m1 - xh * m2)


def kernel(x_ref, wqkv_h, wo_h, wg_h, wu_h, wd_h, dy_ref,
           y_ref, dx_ref, dwqkv_o, dwo_h, dwg_h, dwu_h, dwd_h,
           wqkvT, woT, wgT, wuT, wdT,
           a_qkv, a_o, a_g, a_u, a_d,
           xh1, rs1, xn1, dh_s, h_s, xn2,
           qT, kT, vT, k_s, v_s, dq_s, dk_s, dv_s,
           eb_s, oT, li_s, doT, dl_s,
           s_s, u_s, act, dg_s, du_s, dqkv, sbuf,
           wqkv, wo, wg, wu, wd, dwo_o, dwg_o, dwu_o, dwd_o, sems):
    c = pl.program_id(0)
    slot = c % 2

    cin = [pltpu.make_async_copy(a, b, sems.at[i]) for i, (a, b) in enumerate(
        ((wqkv_h, wqkv), (wo_h, wo), (wg_h, wg), (wu_h, wu), (wd_h, wd)))]
    cout = [pltpu.make_async_copy(a, b, sems.at[5 + i]) for i, (a, b) in enumerate(
        ((dwo_o, dwo_h), (dwg_o, dwg_h), (dwu_o, dwu_h), (dwd_o, dwd_h)))]

    @_when(c == 0, "_init")
    def _init():
        for cp in cin:
            cp.start()
        for a in (a_qkv, a_o, a_g, a_u, a_d, dk_s, dv_s):
            a[...] = jnp.zeros(a.shape, F32)
        cin[0].wait()
        for r, n in _chunks(3 * D, 128):
            wqkvT[r:r + n, :] = wqkv[:, r:r + n].T

    def _init2():
        for cp in cin[1:]:
            cp.wait()
        for r, n in _chunks(D, 128):
            woT[r:r + n, :] = wo[:, r:r + n].T
        for r, n in _chunks(F, 128):
            wgT[:, r:r + n] = wg[r:r + n, :].T
            wuT[:, r:r + n] = wu[r:r + n, :].T
            wdT[:, r:r + n] = wd[r:r + n, :].T

    def _fin1():
        for o, a in ((dwo_o, a_o), (dwg_o, a_g), (dwu_o, a_u), (dwd_o, a_d)):
            o[...] = a[...].astype(BF)
        for cp in cout:
            cp.start()

    kq = jax.lax.broadcasted_iota(jnp.int32, (QB, QB), 0) <= jax.lax.broadcasted_iota(jnp.int32, (QB, QB), 1)

    mk = jnp.where(kq, -1, 0)
    HG = 4

    r2 = jax.lax.broadcasted_iota(jnp.int32, (QB // 2, QB), 0) * 2
    q2 = jax.lax.broadcasted_iota(jnp.int32, (QB // 2, QB), 1)
    m2 = jnp.where(r2 <= q2, 0xFFFF, 0) | jnp.where(r2 + 1 <= q2, -65536, 0)
    pk = lambda v: pltpu.bitcast(v, jnp.int32)
    upk = lambda v: pltpu.bitcast(v, BF)

    def keep(v):
        b = pk(v)
        return upk(b & m2), upk(b & ~m2)

    def head_w(ref, h0, g, j):
        cols = []
        for hh in range(h0, h0 + HG):
            blk = ref[pl.ds(pl.multiple_of((g * HU + hh) * DH, DH), DH), j * QB:(j + 1) * QB]
            lo = hh * DH
            parts = []
            if lo:
                parts.append(jnp.zeros((lo, QB), BF))
            parts.append(blk)
            if QB - lo - DH:
                parts.append(jnp.zeros((QB - lo - DH, QB), BF))
            cols.append(jnp.concatenate(parts, axis=0))
        return jnp.concatenate(cols, axis=1)

    items = [(j, h0) for j in range(2) for h0 in range(0, HU, HG)]

    def geom(first, j):
        nt = min(j + 1, 3) if first else 3
        t0 = 0 if first else 2 * c + j - 2
        return nt, t0

    def scores(first, g, it, tm, wref, buf):
        j, h0 = it
        nt, t0 = geom(first, j)
        kk = tm[pl.ds(pl.multiple_of(t0 * QB, QB), nt * QB), pl.ds(pl.multiple_of(g * 128, 128), 128)]
        s = _nn(kk, head_w(wref, h0, g, j))
        for hh in range(HG):
            o = hh * QB
            sd = s[(nt - 1) * QB:, o:o + QB]
            if nt == 3:
                sd = jnp.where(kq, sd, s[:QB, o:o + QB])
            buf[hh, :QB] = sd
            if nt > 1:
                buf[hh, QB:] = s[(nt - 2) * QB:(nt - 1) * QB, o:o + QB]

    def pipeline(first, tm, wref, consume):
        n, ng = len(items), H // HU
        scores(first, 0, items[0], tm, wref, sbuf.at[0])

        def body(g, carry):
            for i, (j, h0) in enumerate(items):
                gn = g if i + 1 < n else jnp.minimum(g + 1, ng - 1)
                scores(first, gn, items[(i + 1) % n], tm, wref, sbuf.at[(i + 1) % 2])
                for hh in range(HG):
                    consume(first, g, j, h0 + hh, sbuf.at[i % 2, hh])
            return carry
        jax.lax.fori_loop(0, ng, body, 0)

    def fwd_head(first, g, j, hh, sb):
        nt, t0 = geom(first, j)
        h = g * HU + hh
        rows = pl.ds(pl.multiple_of(h * DH, DH), DH)
        sd = sb[:QB]
        if nt < 3:
            sd = jnp.where(kq, sd, -1e30)
        m = sd
        if nt > 1:
            sm = sb[QB:]
            m = jnp.maximum(m, sm)
        m = jnp.max(m, axis=0, keepdims=True)
        ed = jnp.exp2(sd - m)
        l = ed
        pd, po = keep(ed.astype(BF))
        ps = [pd]
        if nt > 1:
            em = jnp.exp2(sm - m)
            l = l + em
            ps = [em.astype(BF)] + ps
        if nt > 2:
            ps = [po] + ps
        p = jnp.concatenate(ps, axis=0)
        eb_s[j, h, :nt * 64] = pk(p)
        vv = jnp.concatenate([vT[t0 + t, rows, :] for t in range(nt)], axis=1)
        li = 1.0 / jnp.sum(l, axis=0, keepdims=True)
        oT[rows, j * QB:(j + 1) * QB] = _nn(vv, p) * li
        li_s[rows, j * QB:(j + 1) * QB] = jnp.broadcast_to(li, (DH, QB))

    def bwd_head(first, g, j, hh, sb):
        nt, t0 = geom(first, j)
        h = g * HU + hh
        rows = pl.ds(pl.multiple_of(h * DH, DH), DH)
        dl = dl_s[pl.ds(pl.multiple_of(h * DH, DH), 8), j * QB:(j + 1) * QB][:1]
        eb = eb_s[j, h, :nt * 64]
        ed = eb[(nt - 1) * 64:]
        if nt > 2:
            ed = ed | eb[:64]
        ed = upk(ed).astype(F32)
        dsd, dso = keep((ed * (sb[:QB] - dl)).astype(BF))
        ds = [dsd]
        if nt > 1:
            ds = [(upk(eb[(nt - 2) * 64:(nt - 1) * 64]).astype(F32) * (sb[QB:] - dl)).astype(BF)] + ds
        if nt > 2:
            ds = [dso] + ds
        ds = jnp.concatenate(ds, axis=0)
        kk = jnp.concatenate([kT[t0 + t, rows, :] for t in range(nt)], axis=1)
        dv = _nt(doT[rows, j * QB:(j + 1) * QB], upk(eb))
        dq_s[slot, rows, j * QB:(j + 1) * QB] = (_nn(kk, ds) * SCALE).astype(BF)
        dk = _nt(qT[rows, j * QB:(j + 1) * QB], ds)
        for t in range(nt):
            dk_s[t0 + t, rows, :] += dk[:, t * QB:(t + 1) * QB]
            dv_s[t0 + t, rows, :] += dv[:, t * QB:(t + 1) * QB]

    attn_fwd = lambda first: pipeline(first, k_s, qT, fwd_head)
    attn_bwd = lambda first: pipeline(first, v_s, doT, bwd_head)

    @_when(c < NC, "_fwd1")
    def _fwd1():
        xt = x_ref[...].astype(F32).T
        h_s[...] = xt
        xh, rs = _ln_t(xt)
        xh1[slot] = xh
        rs1[slot] = jnp.broadcast_to(rs, (8, T))
        xn = xh.astype(BF)
        xn1[slot] = xn
        qT[...] = (_nn(wqkvT[0:D, :], xn) * (SCALE * LOG2E)).astype(BF)
        for wi, tr, tm in ((1, kT, k_s), (2, vT, v_s)):
            r = _nn(wqkvT[wi * D:(wi + 1) * D, :], xn)
            rb = r.astype(BF)
            for j in range(2):
                tr[2 * c + j] = rb[:, j * QB:(j + 1) * QB]
            tm[pl.ds(pl.multiple_of(c * T, T), T), :] = r.T.astype(BF)

    _when(c == 0, "attn_fwdTrue")(lambda: attn_fwd(True))
    _when((c > 0) & (c < NC), "attn_fwdFalse")(lambda: attn_fwd(False))
    _when(c == 0, "_init2")(_init2)

    @_when(c < NC, "_mid")
    def _mid():
        ob = oT[...].astype(BF)
        ht = h_s[...] + _nn(woT[...], ob)
        h_s[...] = ht
        xh2, rs2 = _ln_t(ht)
        xb = xh2.astype(BF)
        xn2[...] = xb
        dy = dy_ref[...]
        dyt = dy.astype(F32).T
        dyb = dyt.astype(BF)
        for r, n in _chunks(F, FC):
            sg = jax.nn.sigmoid(_nn(wg[r:r + n, :], xb))
            u = _nn(wu[r:r + n, :], xb)
            da = _nn(wd[r:r + n, :], dyb)
            act[r:r + n, :] = (sg * u).astype(BF)
            du = da * sg
            du_s[r:r + n, :] = du.astype(BF)
            dg_s[r:r + n, :] = (du * u * (1.0 - sg)).astype(BF)
        y_ref[...] = (h_s[...] + _nn(wdT[...], act[...])).T.astype(BF)
        a_d[...] += _nn(act[...], dy)
        a_g[...] += _nt(dg_s[...], xb)
        a_u[...] += _nt(du_s[...], xb)
        dn = _nn(wgT[...], dg_s[...]) + _nn(wuT[...], du_s[...])
        dht = dyt + _ln_bwd_t(dn, xh2, rs2)
        dh_s[slot] = dht
        dhb = dht.astype(BF)
        a_o[...] += _nt(oT[...].astype(BF), dhb)
        do = _nn(wo[...], dhb) * li_s[...]
        doT[...] = do.astype(BF)
        pr = do * oT[...]
        for h in range(H):
            dl_s[h * DH:h * DH + 8, :] = jnp.broadcast_to(
                jnp.sum(pr[h * DH:(h + 1) * DH], axis=0, keepdims=True), (8, T))

    _when(c == NC - 1, "_fin1")(_fin1)
    _when(c == 0, "attn_bwdTrue")(lambda: attn_bwd(True))
    _when((c > 0) & (c < NC), "attn_bwdFalse")(lambda: attn_bwd(False))

    @_when(c > 0, "_bwd1")
    def _bwd1():
        ps = 1 - slot
        dqkv[0:D, :] = dq_s[ps]
        for j in range(2):
            dqkv[D:2 * D, j * QB:(j + 1) * QB] = (dk_s[2 * c - 2 + j] * (1.0 / LOG2E)).astype(BF)
            dqkv[2 * D:, j * QB:(j + 1) * QB] = dv_s[2 * c - 2 + j].astype(BF)
        a_qkv[...] += _nt(dqkv[...], xn1[ps])
        dn = _nn(wqkv[...], dqkv[...])
        dx_ref[...] = (dh_s[ps] + _ln_bwd_t(dn, xh1[ps], rs1[ps, :1])).T.astype(BF)

    @_when(c == NC, "_fin")
    def _fin():
        for r, n in _chunks(3 * D, 128):
            dwqkv_o[:, r:r + n] = a_qkv[r:r + n, :].T.astype(BF)
        for cp in cout:
            cp.wait()


@jax.jit
def pallas_sequential_preLN__sliding_block__glu_gated_glu__prompt_kernel(
    A_x, A_wqkv, A_wo, B_x, B_w_gate, B_w_up, B_w_down, grad_out,
):
    del B_x
    whole = lambda shape: pl.BlockSpec(shape, lambda c: (0, 0), pipeline_mode=pl.Buffered(1))
    cur = pl.BlockSpec((T, D), lambda c: (jnp.minimum(c, NC - 1), 0))
    prev = pl.BlockSpec((T, D), lambda c: (jnp.maximum(c - 1, 0), 0))
    wshapes = [(D, 3 * D), (D, D), (F, D), (F, D), (F, D)]
    V = pltpu.VMEM
    scratch = [
        V((3 * D, D), BF), V((D, D), BF), V((D, F), BF), V((D, F), BF), V((D, F), BF),
        V((3 * D, D), F32), V((D, D), F32), V((F, D), F32), V((F, D), F32), V((F, D), F32),
        V((2, D, T), F32), V((2, 8, T), F32), V((2, D, T), BF), V((2, D, T), F32), V((D, T), F32), V((D, T), BF),
        V((D, T), BF), V((NB, D, QB), BF), V((NB, D, QB), BF), V((S, D), BF), V((S, D), BF),
        V((2, D, T), BF), V((NB, D, QB), F32), V((NB, D, QB), F32),
        V((2, H, 3 * 64, QB), jnp.int32), V((D, T), F32), V((D, T), F32),
        V((D, T), BF), V((D, T), F32),
        V((8, 128), F32), V((8, 128), F32), V((F, T), BF), V((F, T), BF), V((F, T), BF), V((3 * D, T), BF), V((2, 4, 2 * QB, QB), F32),
    ] + [V(s, BF) for s in wshapes + wshapes[1:]] + [pltpu.SemaphoreType.DMA((9,))]
    hbm = pl.BlockSpec(memory_space=pltpu.MemorySpace.HBM)
    outs = pl.pallas_call(
        kernel,
        grid=(NC + 1,),
        in_specs=[cur] + [hbm] * 5 + [cur],
        out_specs=[cur, prev, whole(wshapes[0])] + [hbm] * 4,
        out_shape=[jax.ShapeDtypeStruct((S, D), BF)] * 2 + [jax.ShapeDtypeStruct(s, BF) for s in wshapes],
        scratch_shapes=scratch,
        compiler_params=pltpu.CompilerParams(
            dimension_semantics=("arbitrary",), vmem_limit_bytes=110 * 1024 * 1024),
    )(A_x.reshape(S, D), A_wqkv, A_wo, B_w_gate.T, B_w_up.T, B_w_down, grad_out.reshape(S, D))
    return (outs[0].reshape(1, S, D), outs[1].reshape(1, S, D), outs[2], outs[3], outs[4].T, outs[5].T, outs[6])
```
